```python
import os as _os
_os.environ.setdefault('JAX_PLATFORMS', 'cpu')
import jax
import jax.numpy as jnp

def _softmax(x, axis=-1):
    return jax.nn.softmax(x, axis=axis)

def _gelu(x):
    return jax.nn.gelu(x, approximate=True)

def _silu(x):
    return jax.nn.silu(x)

def _sigmoid(x):
    return jax.nn.sigmoid(x)

def _layernorm(x, axis=-1, eps=1e-05):
    m = jnp.mean(x, axis=axis, keepdims=True)
    v = jnp.var(x, axis=axis, keepdims=True)
    return (x - m) / jnp.sqrt(v + eps)

def _scatter_add(tgt, idx, src, axis=0):
    return tgt.at[idx].add(src)

def _segment_sum(src, seg, n):
    return jax.ops.segment_sum(src, seg, n)

class _Rng:

    def __init__(self, key):
        self._k = key

    def _next(self):
        self._k, sub = jax.random.split(self._k)
        return sub

    def normal(self, shape):
        return jax.random.normal(self._next(), shape, dtype=jnp.bfloat16)

    def randint(self, lo, hi, shape):
        return jax.random.randint(self._next(), shape, lo, hi, dtype=jnp.int32)

    def uniform(self, shape, lo=0.0, hi=1.0):
        return jax.random.uniform(self._next(), shape, jnp.bfloat16, lo, hi)

    def permutation(self, n):
        return jax.random.permutation(self._next(), n)
kernel_name = 'adaLN_cond__memory_aug_recurrent_mem_tr__moe_arch_mod__prompt'

def setup_inputs():
    _rng = _Rng(jax.random.key(int.from_bytes(__import__("os").urandom(4), "little")))
    _w = lambda a: (lambda t: t.astype(jnp.bfloat16) if jnp.issubdtype(t.dtype, jnp.floating) else t)(jnp.asarray(a))

    def _A_setup():
        B, S, Dm = (1, 2048, 448)
        H, Dh = (16, 256)
        M, seg = (8, 32)
        seg = min(seg, S)
        S = S // seg * seg
        return {'x': _w((lambda *s: _rng.normal(s) * 0.05)(B, S, Dm)), 'mem0': _w((lambda *s: _rng.normal(s) * 0.4)(B, M, Dm)), 'Wq': _w((lambda *s: _rng.normal(s) * 1.6)(Dm, H, Dh) * Dm ** (-0.5)), 'Wk': _w((lambda *s: _rng.normal(s) * 1.6)(Dm, H, Dh) * Dm ** (-0.5)), 'Wv': _w((lambda *s: _rng.normal(s) * 0.4)(Dm, H, Dh) * Dm ** (-0.5)), 'Wo': _w((lambda *s: _rng.normal(s) * 0.4)(H, Dh, Dm) * (H * Dh) ** (-0.5)), 'seg_len': seg}
    _A_in = _A_setup()

    def _B_setup():
        B, S, D, F, C = (1, 2048, 448, 1792, 1)
        return {'x': _w((lambda *s: _rng.normal(s) * 0.05)(B, S, D)), 'w_r': _w((lambda *s: _rng.normal(s) * 0.05)(D)), 'w_gate': _w((lambda *s: _rng.normal(s) * 0.05)(D, F)), 'w_up': _w((lambda *s: _rng.normal(s) * 0.05)(D, F)), 'w_down': _w((lambda *s: _rng.normal(s) * 0.05)(F, D))}
    _B_in = _B_setup()
    return {'A_x': _A_in['x'], 'A_mem0': _A_in['mem0'], 'A_Wq': _A_in['Wq'], 'A_Wk': _A_in['Wk'], 'A_Wv': _A_in['Wv'], 'A_Wo': _A_in['Wo'], 'A_seg_len': _A_in['seg_len'], 'B_x': _B_in['x'], 'B_w_r': _B_in['w_r'], 'B_w_gate': _B_in['w_gate'], 'B_w_up': _B_in['w_up'], 'B_w_down': _B_in['w_down'], 'c': _w((lambda *s: _rng.normal(s) * 0.05)(1, 448) * 8.0), 'w_mod': _w((lambda *s: _rng.normal(s) * 0.05)(448, 6 * 448) * 448 ** (-0.5) * 8.0)}

def reference(A_x, A_mem0, A_Wq, A_Wk, A_Wv, A_Wo, A_seg_len, B_x, B_w_r, B_w_gate, B_w_up, B_w_down, c, w_mod):

    def _A_ref(x, mem0, Wq, Wk, Wv, Wo, seg_len):
        B, S, Dm = x.shape
        H, Dh = (Wq.shape[1], Wq.shape[2])
        M = mem0.shape[1]
        scale = Dh ** (-0.5)
        n_seg = S // seg_len
        L = M + seg_len
        idx = jnp.arange(L)
        mask = (idx[:, None] < M) | (idx[:, None] >= idx[None, :])
        mem = mem0
        outs = []
        for s in range(n_seg):
            xs = x[:, s * seg_len:(s + 1) * seg_len, :].copy()
            h = jnp.concatenate([mem, xs], axis=1)
            q = jnp.einsum('btd,dhe->bhte', h, Wq)
            k = jnp.einsum('btd,dhe->bhte', h, Wk)
            v = jnp.einsum('btd,dhe->bhte', h, Wv)
            scores = jnp.einsum('bhqe,bhke->bhqk', q, k) * scale
            scores = jnp.where(mask[None, None], scores, -1000000000.0)
            p = _softmax(scores, axis=-1)
            o = jnp.einsum('bhqk,bhke->bhqe', p, v)
            o = jnp.einsum('bhte,hed->btd', o, Wo)
            mem = o[:, :M, :].copy()
            outs.append(o[:, M:, :])
        return jnp.concatenate(outs, axis=1)

    def _B_ref(x, w_r, w_gate, w_up, w_down):
        B, S, D = x.shape
        C = 1
        r = x @ w_r
        idx = jnp.argsort(-r, axis=-1)[:, :C]
        idx_e = jnp.repeat(idx.reshape(B, C, 1), D, axis=2)
        x_sel = jnp.take_along_axis(x, idx_e, axis=1)
        g = _silu(x_sel @ w_gate)
        u = x_sel @ w_up
        y = g * u @ w_down
        r_sel = _sigmoid(jnp.take_along_axis(r, idx, axis=1))
        y = y * r_sel.reshape(B, C, 1)
        b_off = (jnp.arange(B) * S).reshape(B, 1)
        flat_idx = (idx + b_off).reshape(B * C)
        zero = (x * 0.0).reshape(B * S, D)
        upd = _scatter_add(zero, flat_idx, y.reshape(B * C, D), axis=0)
        return x + upd.reshape(B, S, D)
    x = A_x
    mod = (_silu(c) @ w_mod).reshape(c.shape[0], 6, 1, -1)
    sa, ca, ga, sb, cb, gb = (mod[:, 0].copy(), mod[:, 1].copy(), mod[:, 2].copy(), mod[:, 3].copy(), mod[:, 4].copy(), mod[:, 5].copy())
    h = _layernorm(x, axis=-1) * (1 + ca) + sa
    x = x + ga * _A_ref(h, A_mem0, A_Wq, A_Wk, A_Wv, A_Wo, A_seg_len)
    h = _layernorm(x, axis=-1) * (1 + cb) + sb
    x = x + gb * _B_ref(h, B_w_r, B_w_gate, B_w_up, B_w_down)
    return x
```

```python
import functools

import jax
import jax.numpy as jnp
from jax import lax
import jax.experimental.pallas as pl
import jax.experimental.pallas.tpu as pltpu

D = 448
DM = 384
DT = D - DM
DP = 512
NH = 16
NP = NH // 2
DH = 256
NM = 8
SEG = 32
L = NM + SEG
NB = L // 8
S = 2048
NSEG = S // SEG
NG = S // 128
FF = 1792
EPS = 1e-5

_EDGES = dict(wv=(0, 128, 288, D), wq=(0, 128, 256, D), wk=(0, 128, 256, D))
_GROUPS = [[("w" + t[0], int(t[1])) for t in g.split()] for g in
           "o0 v0|v1|o1|o2|o3|o4 o5|o6 o7|v2|q0 k0 q1|k1|k2|q2".split("|")]
_ARRIVALS = tuple(a for g in _GROUPS for a in g) + (
    ("w", 0), ("x", 0), ("x", 1), ("w", 1), ("w", 2), ("w", 3))
_AHEAD = 8
_NSEM = sum(1 if k in ("wo", "w") else 2 for k, _ in _ARRIVALS) + 3

F32 = jnp.float32
BF16 = jnp.bfloat16
U32 = jnp.uint32
NN = (((1,), (0,)), ((), ()))
NT = (((1,), (1,)), ((), ()))


def _dot(a, b, dims=NN):
    return lax.dot_general(a, b, dims, preferred_element_type=F32)


def _pack(x):
    return pltpu.bitcast(x.astype(BF16), U32)


def _unpack(x):
    return pltpu.bitcast(x, BF16)


def _lane(shape):
    return lax.broadcasted_iota(jnp.int32, shape, 1)


def _widen(v):
    t = v[:, DM:D]
    return jnp.concatenate([v[:, :DM], t, t], axis=1)


def _feat_sum(v):
    head = _lane((v.shape[0], 128)) < DT
    acc = v[:, 0:128] + v[:, 128:256] + v[:, 256:384] + jnp.where(head, v[:, 384:512], 0.0)
    return jnp.sum(acc, axis=1, keepdims=True)


def _norm_mod(v, scale1, shift):
    xc = v - _feat_sum(v) * (1.0 / D)
    var = _feat_sum(xc * xc) * (1.0 / D)
    return xc * lax.rsqrt(var + EPS) * scale1 + shift


def _group8(x, op):
    lane = _lane(x.shape)
    for s in (1, 2, 4):
        partner = jnp.where((lane & s) == 0, pltpu.roll(x, 128 - s, 1), pltpu.roll(x, s, 1))
        x = op(x, partner)
    return x


def _head_pair(buf, p, r0, r1):
    rows = pl.ds(r0 * NP + p, r1 - r0, stride=NP)
    u = jnp.concatenate([buf.at[t].bitcast(U32)[rows, :] for t in range(2)], axis=1)
    lo = pltpu.bitcast(u << 16, F32)
    hi = pltpu.bitcast(u & jnp.uint32(0xFFFF0000), F32)
    return lo, hi


def _merge_main(lhs, rhs, scale, wm_ref, p, d0, d1, e0, e1):
    for i in range(2):
        a = _dot(lhs[i], rhs[i], NT)
        if scale != 1.0:
            a = a * scale
        for j in range(e0 // 128, e1 // 128):
            wm_ref[j, p, d0 // 2:d1 // 2, i * 128:(i + 1) * 128] = _pack(
                a[:, j * 128 - e0:(j + 1) * 128 - e0])


def _merge_tail(lhs, rhs_tail, scale, wt_ref, p):
    z = jnp.zeros((DT, DH), BF16)
    a = jnp.concatenate(
        [_dot(rhs_tail[i], jnp.concatenate([lhs[i].astype(BF16), z], axis=0), NT)
         for i in range(2)], axis=0)
    if scale != 1.0:
        a = a * scale
    wt_ref[p] = _pack(a.T)


def _project_main(hm, wm_ref, st_ref, j, p):
    y = _dot(hm, _unpack(wm_ref[j, p]))
    for kb in range(NB):
        r = y[kb * 8:(kb + 1) * 8]
        blk = jnp.concatenate([r[:, :128], r[:, 128:]], axis=0)
        st_ref[kb * 64 + p * 8:kb * 64 + p * 8 + 8, j * 128:(j + 1) * 128] = _pack(blk)


def _project_tail(hm, wt_ref, st_ref, p, dup):
    head = _lane((8, 128)) < DT
    y = _dot(hm, _unpack(wt_ref[p]))
    other = pltpu.roll(y, DT, 1) if dup else jnp.zeros_like(y)
    for kb in range(NB):
        r, o = y[kb * 8:(kb + 1) * 8], other[kb * 8:(kb + 1) * 8]
        blk = jnp.concatenate([jnp.where(head, r, o), jnp.where(head, o, r)], axis=0)
        st_ref[kb * 64 + p * 8:kb * 64 + p * 8 + 8, DM:DP] = _pack(blk)


def _seeing(kb):
    return [0] + list(range(max(kb, 1), NB))


def _scores(hq, ys_ref, kb):
    qbs = _seeing(kb)
    sc = _dot(jnp.concatenate([hq[q] for q in qbs], axis=0),
              _unpack(ys_ref[kb * 64:(kb + 1) * 64, :]), NT)
    return {q: sc[i * 8:(i + 1) * 8] for i, q in enumerate(qbs)}


def _softmax(sc):
    tri = (_lane((8, 128)) & 7) <= lax.broadcasted_iota(jnp.int32, (8, 128), 0)
    vis = [{kb: jnp.where(tri, sc[kb][qb], -1e9) if 0 < qb == kb else sc[kb][qb]
            for kb in range(NB) if qb in sc[kb]} for qb in range(NB)]
    mx = _group8(jnp.concatenate(
        [functools.reduce(jnp.maximum, r.values()) for r in vis], axis=0), jnp.maximum)
    ex = [{kb: jnp.exp(t - mx[qb * 8:(qb + 1) * 8]) for kb, t in r.items()}
          for qb, r in enumerate(vis)]
    den = _group8(jnp.concatenate(
        [functools.reduce(jnp.add, r.values()) for r in ex], axis=0), jnp.add)
    inv = 1.0 / den
    return [{kb: t * inv[qb * 8:(qb + 1) * 8] for kb, t in r.items()} for qb, r in enumerate(ex)]


def _attend(prob, fs_ref, j):
    acc = [None] * NB
    for kb in (0, 1, 2, 3, 4) if j == 2 else (0, 4, 1, 3, 2):
        qbs = _seeing(kb)
        o = _dot(jnp.concatenate([prob[q][kb] for q in qbs], axis=0),
                 _unpack(fs_ref[kb * 64:(kb + 1) * 64, j * 128:(j + 1) * 128]))
        for i, q in enumerate(qbs):
            t = o[i * 8:(i + 1) * 8]
            acc[q] = t if acc[q] is None else acc[q] + t
    return jnp.concatenate(acc, axis=0)


def _kernel(xT_hbm, mem0_ref, wq_hbm, wk_hbm, wv_hbm, woT_hbm, wr_ref, wg_hbm, wu_hbm, wdT_hbm,
            c_ref, wmod_hbm, out_hbm,
            xT_v, wq_v, wk_v, wv_v, woT_v, wmod_v, wg_v, wu_v, wd_v,
            wym, wyt, wfm, wft, ys, fs, vec, xtok, hbuf, obuf, h2tok, ztok, outT_v, sems):
    def copy(i, src, dst):
        return pltpu.make_async_copy(src, dst, sems.at[i])

    plan = []
    for kind, i in _ARRIVALS:
        if kind == "wo":
            pairs = [(woT_hbm.at[pl.ds(2 * i, 2)], woT_v.at[pl.ds(2 * i, 2)])]
        elif kind in ("wv", "wq", "wk"):
            src, dst = {"wv": (wv_hbm, wv_v), "wq": (wq_hbm, wq_v), "wk": (wk_hbm, wk_v)}[kind]
            r = pl.ds(_EDGES[kind][i] * NH, (_EDGES[kind][i + 1] - _EDGES[kind][i]) * NH)
            pairs = [(src.at[r, pl.ds(t * 128, 128)], dst.at[t, r]) for t in range(2)]
        elif kind == "x":
            cols = pl.ds(0, 512) if i == 0 else pl.ds(512, S - 512)
            pairs = [(xT_hbm.at[:, cols], xT_v.at[pl.ds(0, D), cols]),
                     (xT_hbm.at[pl.ds(DM, DT), cols], xT_v.at[pl.ds(D, DT), cols])]
        else:
            pairs = [[(wmod_hbm, wmod_v), (wg_hbm, wg_v), (wu_hbm, wu_v), (wdT_hbm, wd_v)][i]]
        first = sum(len(c) for c in plan)
        plan.append([copy(first + n, a, b) for n, (a, b) in enumerate(pairs)])
    started = 0

    def arrive(kind, i):
        nonlocal started
        n = _ARRIVALS.index((kind, i))
        while started < min(n + 1 + _AHEAD, len(plan)):
            for c in plan[started]:
                c.start()
            started += 1
        for c in plan[n]:
            c.wait()

    for pieces in plan[:_AHEAD]:
        for c in pieces:
            c.start()
    started = _AHEAD

    for wm_ref, wt_ref in ((wym, wyt), (wfm, wft)):
        wm_ref[:, :, D // 2:, :] = jnp.zeros((3, NP, DT // 2, 256), U32)
    obuf[...] = jnp.zeros(obuf.shape, F32)
    ztok[0:128, :] = jnp.zeros((128, DP), F32)

    def merge_f(p, d0, d1):
        wo = [woT_v[2 * p + i, 0:DM, :] for i in range(2)]
        _merge_main(_head_pair(wv_v, p, d0, d1), wo, 1.0, wfm, p, d0, d1, 0, DM)

    def merge_y(p, d0, d1, e0, e1):
        e1 = min(e1, DM)
        if e0 < e1 and d0 < d1:
            q = [t.astype(BF16) for t in _head_pair(wq_v, p, e0, e1)]
            _merge_main(_head_pair(wk_v, p, d0, d1), q, DH ** -0.5, wym, p, d0, d1, e0, e1)

    def rows(i):
        return jnp.concatenate([vec[i]] * (SEG // 8), axis=0)

    def x_tile(g, j):
        g0, j0 = pl.multiple_of(g * 128, 128), pl.multiple_of(j * 128, 128)
        t = xT_v[pl.ds(j0, 128), pl.ds(g0, 128)].astype(F32).T
        xtok[pl.ds(g0, 128), pl.ds(j0, 128)] = t
        return t[120:128]

    def out_tile(g, j):
        g0, j0 = pl.multiple_of(g * 128, 128), pl.multiple_of(j * 128, 128)
        t = ztok[pl.ds(g0, 128), pl.ds(j0, 128)].T
        outT_v[pl.ds(j0, 128), pl.ds(g0, 128)] = t.astype(BF16)
        return t[120:128]

    def seg_rows(s):
        return pl.ds(pl.multiple_of(s * SEG, SEG), SEG)

    def pre(s):
        h = _norm_mod(xtok[seg_rows(s), :], rows(1), rows(0))
        hbuf[...] = h
        return functools.reduce(jnp.maximum, [h[b * 8:(b + 1) * 8, 0:128] for b in range(SEG // 8)])

    def post(s, live, best, bidx):
        x1 = xtok[seg_rows(s), :] + rows(2) * obuf[...]
        h2 = _norm_mod(x1, rows(4), rows(3))
        h2tok[seg_rows(s), :] = h2
        ztok[seg_rows(s), :] = x1 + rows(5) * h2
        r = _feat_sum(h2 * rows(6))
        sub = lax.broadcasted_iota(jnp.int32, (8, 128), 0)
        for b in range(SEG // 8):
            rb = jnp.broadcast_to(r[b * 8:(b + 1) * 8], (8, 128))
            better = jnp.logical_and(rb > best, live)
            best = jnp.where(better, rb, best)
            bidx = jnp.where(better, sub + (s * SEG + b * 8), bidx)
        return best, bidx

    def setup():
        arrive("w", 0)
        arrive("x", 0)
        cv = jnp.broadcast_to(c_ref[...].astype(F32), (8, D))
        mod = _dot(cv * jax.nn.sigmoid(cv), wmod_v[...])
        for i in range(6):
            v = _widen(mod[:, i * D:(i + 1) * D])
            vec[i] = v + 1.0 if i in (1, 4) else v
        vec[6] = _widen(jnp.broadcast_to(wr_ref[...].astype(F32).reshape(1, D), (8, D)))
        for g in range(2):
            for j in range(4):
                x_tile(g, j)
        pre(0)

    have = dict(wo=0, wv=0, wq=0, wk=0)
    ev, eq, ek = _EDGES["wv"], _EDGES["wq"], _EDGES["wk"]
    for group in _GROUPS:
        old = dict(have)
        for kind, i in group:
            arrive(kind, i)
            have[kind] += 1
        for p in range(have["wo"]):
            d0, d1 = ev[old["wv"]] if p < old["wo"] else 0, ev[have["wv"]]
            if d0 < d1:
                merge_f(p, d0, d1)
                if d1 == D:
                    _merge_tail(_head_pair(wv_v, p, 0, D),
                                [woT_v[2 * p + i, DM:D, :] for i in range(2)], 1.0, wft, p)
        for p in range(NP):
            if group is _GROUPS[-1] and p == 6:
                setup()
            merge_y(p, ek[old["wk"]], ek[have["wk"]], 0, eq[old["wq"]])
            merge_y(p, 0, ek[have["wk"]], eq[old["wq"]], eq[have["wq"]])
            if (ek[have["wk"]], eq[have["wq"]]) == (D, D) != (ek[old["wk"]], eq[old["wq"]]):
                _merge_tail(_head_pair(wk_v, p, 0, D), _head_pair(wq_v, p, DM, D), DH ** -0.5,
                            wyt, p)

    n_early = NG - 2
    early = copy(_NSEM - 3, outT_v.at[pl.ds(0, D), pl.ds(0, n_early * 128)],
                 out_hbm.at[:, pl.ds(0, n_early * 128)])

    def step(s, carry):
        mem, best, bidx = carry
        pl.when(s == 8)(lambda: arrive("x", 1))
        pl.when(s == NSEG - 2)(early.start)
        hm = jnp.concatenate([mem, hbuf[...]], axis=0)
        hq = [hm[q * 8:(q + 1) * 8] for q in range(NB)]
        best, bidx = post(jnp.maximum(s - 1, 0), s > 0, best, bidx)

        def after(dep):
            first = jnp.where(s < 0, dep, hm[NM:NM + 8, 0:128])
            row = jnp.concatenate([first, hm[NM:NM + 8, 128:]], axis=1)
            return jnp.concatenate([hm[:NM], row, hm[NM + 8:]], axis=0)

        t = jnp.maximum(s - 5, 0)
        side = [best, pre(jnp.minimum(s + 1, NSEG - 1)),
                x_tile(jnp.minimum(s // 4 + 2, NG - 1), s % 4), out_tile(t // 4, t % 4)]
        for j in range(3):
            for p in range(NP):
                k = j * NP + p
                lhs = after(side[(k - 8) // 4]) if k in (8, 12, 16, 20) else hm
                _project_main(lhs, wym, ys, j, p)
        for p in range(NP):
            _project_tail(hm, wyt, ys, p, False)
        sc = {}
        for p in range(NP):
            _project_tail(hm, wft, fs, p, True)
            if p in (3, 7):
                sc[len(sc)] = _scores(hq, ys, len(sc))
        for j in range(3):
            for p in range(NP):
                _project_main(hm, wfm, fs, j, NP - 1 - p if j == 2 else p)
                if j * NP + p in (1, 4, 7):
                    sc[len(sc)] = _scores(hq, ys, len(sc))
        prob = _softmax(sc)
        o = {j: _attend(prob, fs, j) for j in (3, 0, 1, 2)}
        o = jnp.concatenate([o[j] for j in range(4)], axis=1)
        obuf[...] = o[NM:]
        return o[:NM], best, bidx

    init = (_widen(mem0_ref[...].astype(F32)),
            jnp.full((8, 128), -jnp.inf, F32), jnp.zeros((8, 128), jnp.int32))
    _, best, bidx = lax.fori_loop(0, NSEG, step, init)
    for i in (1, 2, 3):
        arrive("w", i)
    early.wait()
    best, bidx = post(NSEG - 1, True, best, bidx)

    top = jnp.max(best, axis=0, keepdims=True)
    idx = jnp.min(jnp.where(best == top, bidx, S - 1))
    sel = jnp.broadcast_to(h2tok[pl.ds(idx, 1), :], (8, DP))[:, :D]
    gate = _dot(sel, wg_v[...])
    act = gate * jax.nn.sigmoid(gate) * _dot(sel, wu_v[...])
    y = _widen(_dot(act, wd_v[...], NT)) * jax.nn.sigmoid(top[:, 0:1])
    ztok[pl.ds(idx, 1), :] = ztok[pl.ds(idx, 1), :] + (vec[5] * y)[0:1]

    top_g = idx // 128
    out_tile(NG - 2, 3)
    for j in range(4):
        out_tile(NG - 1, j)
        out_tile(top_g, j)
    rest = pl.ds(n_early * 128, S - n_early * 128)
    last = copy(_NSEM - 2, outT_v.at[pl.ds(0, D), rest], out_hbm.at[:, rest])
    last.start()

    @pl.when(top_g < n_early)
    def _():
        cols = pl.ds(pl.multiple_of(top_g * 128, 128), 128)
        patch = copy(_NSEM - 1, outT_v.at[pl.ds(0, D), cols], out_hbm.at[:, cols])
        patch.start()
        patch.wait()

    last.wait()


@functools.partial(jax.jit, static_argnames=("A_seg_len",))
def pallas_adaLN_cond__memory_aug_recurrent_mem_tr__moe_arch_mod__prompt_kernel(
    A_x: jax.Array,
    A_mem0: jax.Array,
    A_Wq: jax.Array,
    A_Wk: jax.Array,
    A_Wv: jax.Array,
    A_Wo: jax.Array,
    A_seg_len: int,
    B_x: jax.Array,
    B_w_r: jax.Array,
    B_w_gate: jax.Array,
    B_w_up: jax.Array,
    B_w_down: jax.Array,
    c: jax.Array,
    w_mod: jax.Array,
):
    del B_x
    assert A_seg_len == SEG and A_x.shape == (1, S, D) and A_Wq.shape == (D, NH, DH)
    hbm = pl.BlockSpec(memory_space=pl.ANY)
    vmem = pl.BlockSpec(memory_space=pltpu.VMEM)
    split = pltpu.VMEM((2, D * NH, 128), BF16)
    wmain = pltpu.VMEM((3, NH // 2, DP // 2, 256), U32)
    wtail = pltpu.VMEM((NH // 2, DP // 2, 128), U32)
    stack = pltpu.VMEM((NB * 64, DP), U32)
    tok = pltpu.VMEM((S, DP), F32)
    ff = pltpu.VMEM((D, FF), BF16)
    outT = pl.pallas_call(
        _kernel,
        out_shape=jax.ShapeDtypeStruct((D, S), BF16),
        in_specs=[hbm, vmem, hbm, hbm, hbm, hbm, vmem, hbm, hbm, hbm, vmem, hbm],
        out_specs=hbm,
        scratch_shapes=[
            pltpu.VMEM((DP, S), BF16), split, split, split, pltpu.VMEM((NH, D, DH), BF16),
            pltpu.VMEM((D, 6 * D), BF16), ff, ff, ff,
            wmain, wtail, wmain, wtail, stack, stack, pltpu.VMEM((7, 8, DP), F32),
            tok, pltpu.VMEM((SEG, DP), F32), pltpu.VMEM((SEG, DP), F32), tok, tok,
            pltpu.VMEM((DP, S), BF16), pltpu.SemaphoreType.DMA((_NSEM,)),
        ],
        compiler_params=pltpu.CompilerParams(vmem_limit_bytes=100 * 1024 * 1024),
    )(
        A_x[0].T, A_mem0[0],
        A_Wq.reshape(D * NH, DH), A_Wk.reshape(D * NH, DH), A_Wv.reshape(D * NH, DH),
        A_Wo.transpose(0, 2, 1), B_w_r, B_w_gate, B_w_up, B_w_down.T, c, w_mod,
    )
    return outT.T[None]
```

```python
import functools

import jax
import jax.numpy as jnp
from jax import lax
import jax.experimental.pallas as pl
import jax.experimental.pallas.tpu as pltpu

D = 448
DM = 384
DT = D - DM
DP = 512
NH = 16
NP = NH // 2
DH = 256
NM = 8
SEG = 32
L = NM + SEG
NB = L // 8
S = 2048
NSEG = S // SEG
NG = S // 128
FF = 1792
EPS = 1e-5
SCALE = DH ** -0.5

_EDGES = (0, 128, 256, DM, D)
_GROUPS = [[("w" + t[0], int(t[1])) for t in g.split()] for g in
           "o0 v0|v1|o1|v3|o2|o3|o4 o5|o6 o7|v2|q0 k0 q1|k1|q3 k3|q2|k2".split("|")]
_ARRIVALS = tuple(a for g in _GROUPS for a in g) + (
    ("w", 0), ("x", 0), ("x", 1), ("x", 2), ("w", 1))
_AHEAD = 8
_NSEM = sum({"wo": 1, "w": 4}.get(k, 2) for k, _ in _ARRIVALS) + 3

_UNROLL = 4
_TILES = (3, 0, 1, 2)

F32 = jnp.float32
BF16 = jnp.bfloat16
U32 = jnp.uint32
NN = (((1,), (0,)), ((), ()))
NT = (((1,), (1,)), ((), ()))


def _dot(a, b, dims=NN):
    return lax.dot_general(a, b, dims, preferred_element_type=F32)


def _pack(x):
    return pltpu.bitcast(x.astype(BF16), U32)


def _unpack(x):
    return pltpu.bitcast(x, BF16)


def _lane(shape):
    return lax.broadcasted_iota(jnp.int32, shape, 1)


def _widen(v):
    t = v[:, DM:D]
    return jnp.concatenate([v[:, :DM], t, t], axis=1)


def _feat_sum(v):
    head = _lane((v.shape[0], 128)) < DT
    acc = v[:, 0:128] + v[:, 128:256] + v[:, 256:384] + jnp.where(head, v[:, 384:512], 0.0)
    return jnp.sum(acc, axis=1, keepdims=True)


def _norm_mod(v, scale1, shift):
    xc = v - _feat_sum(v) * (1.0 / D)
    var = _feat_sum(xc * xc) * (1.0 / D)
    return xc * lax.rsqrt(var + EPS) * scale1 + shift


def _group8(x, op):
    lane = _lane(x.shape)
    for size, step in ((4, 1), (8, 4)):
        pos = lane & (size - 1)
        x = functools.reduce(op, [x] + [
            jnp.where(pos >= d, pltpu.roll(x, d, 1), pltpu.roll(x, 128 + d - size, 1))
            for d in range(step, size, step)])
    return x


def _head_pair(buf, p, i):
    rows = pl.ds(_EDGES[i] * NP + p, _EDGES[i + 1] - _EDGES[i], stride=NP)
    u = jnp.concatenate([buf.at[t].bitcast(U32)[rows, :] for t in range(2)], axis=1)
    lo = pltpu.bitcast(u << 16, F32)
    hi = pltpu.bitcast(u & jnp.uint32(0xFFFF0000), F32)
    return lo, hi


def _merge_tail(lhs_tail, rhs, scale):
    pad = [jnp.zeros((128 - rhs[0].shape[0], DH), BF16)] if rhs[0].shape[0] < 128 else []
    a = jnp.concatenate(
        [_dot(lhs_tail[h], jnp.concatenate([rhs[h].astype(BF16)] + pad, axis=0), NT)
         for h in range(2)], axis=0)
    return _pack((a if scale == 1.0 else a * scale).T)


def _project_main(hm, wm_ref, st_ref, j, p):
    y = _dot(hm, _unpack(wm_ref[j, p]))
    for kb in range(NB):
        r = y[kb * 8:(kb + 1) * 8]
        blk = jnp.concatenate([r[:, :128], r[:, 128:]], axis=0)
        st_ref[kb * 64 + p * 8:kb * 64 + p * 8 + 8, j * 128:(j + 1) * 128] = _pack(blk)


def _project_tail(hm, wt_ref, st_ref, p, dup):
    head = _lane((8, 128)) < DT
    y = _dot(hm, _unpack(wt_ref[p]))
    other = pltpu.roll(y, DT, 1) if dup else jnp.zeros_like(y)
    for kb in range(NB):
        r, o = y[kb * 8:(kb + 1) * 8], other[kb * 8:(kb + 1) * 8]
        blk = jnp.concatenate([jnp.where(head, r, o), jnp.where(head, o, r)], axis=0)
        st_ref[kb * 64 + p * 8:kb * 64 + p * 8 + 8, DM:DP] = _pack(blk)


def _seeing(kb):
    return [0] + list(range(max(kb, 1), NB))


def _scores(hq, ys_ref, kb):
    qbs = _seeing(kb)
    sc = _dot(jnp.concatenate([hq[q] for q in qbs], axis=0),
              _unpack(ys_ref[kb * 64:(kb + 1) * 64, :]), NT)
    return {q: sc[i * 8:(i + 1) * 8] for i, q in enumerate(qbs)}


def _tail_keys(hq):
    head = _lane((8, 128)) < DT
    blk = [jnp.concatenate([jnp.where(head, t[:, DM:], 0.0), jnp.where(head, 0.0, t[:, DM:])],
                           axis=0).astype(BF16) for t in hq]
    blk += [jnp.zeros((16, 128), BF16)] * (NP - NB)
    return [jnp.concatenate([blk[(i - p) % NP] for i in range(NP)], axis=0) for p in range(NP)]


def _add_tail_scores(sc, st):
    slot = _lane((8, 128)) // 16
    out = {}
    for kb in range(NB):
        out[kb] = {}
        for qb in sc[kb]:
            g = st[0][qb * 8:(qb + 1) * 8]
            for p in range(1, NP):
                g = jnp.where(slot == (p + kb) % NP, st[p][qb * 8:(qb + 1) * 8], g)
            out[kb][qb] = sc[kb][qb] + (pltpu.roll(g, 128 - 16 * kb, 1) if kb else g)
    return out


def _slot_probs(prob):
    slot = _lane((8, 128)) // 16
    rot = [{kb: pltpu.roll(t, 16 * kb, 1) if kb else t for kb, t in r.items()} for r in prob]
    out = []
    for p in range(NP):
        rows = []
        for r in rot:
            g = r[0] if len(r) == NB else jnp.where(slot == p, r[0], 0.0)
            for kb in range(1, len(r)):
                g = jnp.where(slot == (p + kb) % NP, r[kb], g)
            rows.append(g)
        out.append(jnp.concatenate(rows, axis=0))
    return out


def _softmax(sc):
    tri = (_lane((8, 128)) & 7) <= lax.broadcasted_iota(jnp.int32, (8, 128), 0)
    vis = [{kb: jnp.where(tri, sc[kb][qb], -1e9) if 0 < qb == kb else sc[kb][qb]
            for kb in range(NB) if qb in sc[kb]} for qb in range(NB)]
    mx = _group8(jnp.concatenate(
        [functools.reduce(jnp.maximum, r.values()) for r in vis], axis=0), jnp.maximum)
    ex = [{kb: jnp.exp(t - mx[qb * 8:(qb + 1) * 8]) for kb, t in r.items()}
          for qb, r in enumerate(vis)]
    den = _group8(jnp.concatenate(
        [functools.reduce(jnp.add, r.values()) for r in ex], axis=0), jnp.add)
    inv = 1.0 / den
    return [{kb: t * inv[qb * 8:(qb + 1) * 8] for kb, t in r.items()} for qb, r in enumerate(ex)]


def _attend(prob, fs_ref, j):
    acc = [None] * NB
    for kb in range(NB):
        qbs = _seeing(kb)
        o = _dot(jnp.concatenate([prob[q][kb] for q in qbs], axis=0),
                 _unpack(fs_ref[kb * 64:(kb + 1) * 64, j * 128:(j + 1) * 128]))
        for i, q in enumerate(qbs):
            t = o[i * 8:(i + 1) * 8]
            acc[q] = t if acc[q] is None else acc[q] + t
    return jnp.concatenate(acc, axis=0)


def _kernel(xT_hbm, mem0_hbm, wq_hbm, wk_hbm, wv_hbm, woT_hbm, wr_hbm, wg_hbm, wu_hbm, wdT_hbm,
            c_hbm, wmod_hbm, out_hbm,
            xT_v, wq_v, wk_v, wv_v, woT_v, wmod_v, wg_v, wu_v, wd_v,
            wym, wyt, wyq, wfm, wft, wfu, ys, fs, vec, xtok, hbuf, obuf, h2tok, ztok, outT_v,
            mem0_ref, wr_ref, c_ref, sems):
    def copy(i, src, dst):
        return pltpu.make_async_copy(src, dst, sems.at[i])

    plan = []
    for kind, i in _ARRIVALS:
        if kind == "wo":
            pairs = [(woT_hbm.at[pl.ds(2 * i, 2)], woT_v.at[pl.ds(2 * i, 2)])]
        elif kind in ("wv", "wq", "wk"):
            src, dst = {"wv": (wv_hbm, wv_v), "wq": (wq_hbm, wq_v), "wk": (wk_hbm, wk_v)}[kind]
            r = pl.ds(_EDGES[i] * NH, (_EDGES[i + 1] - _EDGES[i]) * NH)
            pairs = [(src.at[r, pl.ds(t * 128, 128)], dst.at[t, r]) for t in range(2)]
        elif kind == "x":
            cols = pl.ds(*((0, 256), (256, 256), (512, S - 512))[i])
            pairs = [(xT_hbm.at[:, cols], xT_v.at[pl.ds(0, D), cols]),
                     (xT_hbm.at[pl.ds(DM, DT), cols], xT_v.at[pl.ds(D, DT), cols])]
        else:
            pairs = [[(mem0_hbm, mem0_ref), (wr_hbm, wr_ref), (c_hbm, c_ref), (wmod_hbm, wmod_v)],
                     [(wg_hbm, wg_v), (wu_hbm, wu_v), (wdT_hbm, wd_v)]][i]
        first = sum(len(c) for c in plan)
        plan.append([copy(first + n, a, b) for n, (a, b) in enumerate(pairs)])
    started = 0

    def arrive(kind, i):
        nonlocal started
        n = _ARRIVALS.index((kind, i))
        while started < min(n + 1 + _AHEAD, len(plan)):
            for c in plan[started]:
                c.start()
            started += 1
        for c in plan[n]:
            c.wait()

    for pieces in plan[:_AHEAD]:
        for c in pieces:
            c.start()
    started = _AHEAD

    obuf[...] = jnp.zeros(obuf.shape, F32)
    ztok[0:128, :] = jnp.zeros((128, DP), F32)

    def merge_f(p, i):
        v, rows = _head_pair(wv_v, p, i), slice(i * 64, (i + 1) * 64)
        wo = [woT_v[2 * p + h, 0:DM, :] for h in range(2)]
        wo_tail = [woT_v[2 * p + h, DM:D, :] for h in range(2)]
        for h in range(2):
            if i < 3:
                a = _dot(v[h], wo[h], NT)
                for j in range(3):
                    wfm[j, p, rows, h * 128:(h + 1) * 128] = _pack(a[:, j * 128:(j + 1) * 128])
            else:
                a = _dot(v[h], jnp.concatenate([wo[h], wo_tail[h], wo_tail[h]], axis=0), NT)
                for j in range(4):
                    wfu[j, p * 64 + h * 32:p * 64 + h * 32 + 32, :] = _pack(
                        a[:, j * 128:(j + 1) * 128])
        if i < 3:
            wft[p, rows, :] = _merge_tail(wo_tail, v, 1.0)

    def merge_y(p, i, j):
        k, q = _head_pair(wk_v, p, i), _head_pair(wq_v, p, j)
        if i == 3:
            wyq[p // 2, j * 64:(j + 1) * 64, (p % 2) * 128:(p % 2 + 1) * 128] = _merge_tail(
                k, q, SCALE)
        elif j == 3:
            wyt[p, i * 64:(i + 1) * 64, :] = _merge_tail(q, k, SCALE)
        else:
            for h in range(2):
                wym[j, p, i * 64:(i + 1) * 64, h * 128:(h + 1) * 128] = _pack(
                    _dot(k[h], q[h].astype(BF16), NT) * SCALE)

    def rows(i):
        return jnp.concatenate([vec[i]] * (SEG // 8), axis=0)

    def x_tile(g, j):
        g0, j0 = pl.multiple_of(g * 128, 128), pl.multiple_of(j * 128, 128)
        t = xT_v[pl.ds(j0, 128), pl.ds(g0, 128)].astype(F32).T
        xtok[pl.ds(g0, 128), pl.ds(j0, 128)] = t
        return t[120:128]

    def out_tile(g, j):
        g0, j0 = pl.multiple_of(g * 128, 128), pl.multiple_of(j * 128, 128)
        t = ztok[pl.ds(g0, 128), pl.ds(j0, 128)].T
        outT_v[pl.ds(j0, 128), pl.ds(g0, 128)] = t.astype(BF16)
        return t[120:128]

    def seg_rows(s):
        return pl.ds(pl.multiple_of(s * SEG, SEG), SEG)

    def pre(s):
        h = _norm_mod(xtok[seg_rows(s), :], rows(1), rows(0))
        hbuf[...] = h
        return functools.reduce(jnp.maximum, [h[b * 8:(b + 1) * 8, 0:128] for b in range(SEG // 8)])

    def post(s, live, best, bidx):
        x1 = xtok[seg_rows(s), :] + rows(2) * obuf[...]
        h2 = _norm_mod(x1, rows(4), rows(3))
        h2tok[seg_rows(s), :] = h2
        ztok[seg_rows(s), :] = x1 + rows(5) * h2
        r = _feat_sum(h2 * rows(6))
        sub = lax.broadcasted_iota(jnp.int32, (8, 128), 0)
        for b in range(SEG // 8):
            rb = jnp.broadcast_to(r[b * 8:(b + 1) * 8], (8, 128))
            better = jnp.logical_and(rb > best, live)
            best = jnp.where(better, rb, best)
            bidx = jnp.where(better, sub + (s * SEG + b * 8), bidx)
        return best, bidx

    def setup():
        arrive("w", 0)
        arrive("x", 0)
        cv = jnp.broadcast_to(c_ref[...].astype(F32), (8, D))
        mod = _dot(cv * jax.nn.sigmoid(cv), wmod_v[...])
        for i in range(6):
            v = _widen(mod[:, i * D:(i + 1) * D])
            vec[i] = v + 1.0 if i in (1, 4) else v
        vec[6] = _widen(jnp.broadcast_to(wr_ref[...].astype(F32).reshape(1, D), (8, D)))
        for g in range(2):
            for j in range(4):
                x_tile(g, j)
        pre(0)

    have = []
    for group in _GROUPS:
        for piece in group:
            arrive(*piece)
        have += group

        def fresh(a, b):
            return a in have and b in have and (a in group or b in group)

        for p in range(NP):
            if group is _GROUPS[-1] and p == 6:
                setup()
            for i in range(4):
                if fresh(("wv", i), ("wo", p)):
                    merge_f(p, i)
                for j in range(4):
                    if fresh(("wk", i), ("wq", j)):
                        merge_y(p, i, j)

    arrive("x", 1)
    s_early = NSEG - _UNROLL
    n_early = (s_early - 9) // 4 + 1
    early = copy(_NSEM - 3, outT_v.at[pl.ds(0, D), pl.ds(0, n_early * 128)],
                 out_hbm.at[:, pl.ds(0, n_early * 128)])

    def step(s, carry):
        mem, best, bidx = carry
        hm = jnp.concatenate([mem, hbuf[...]], axis=0)
        hq = [hm[q * 8:(q + 1) * 8] for q in range(NB)]
        best, bidx = post(jnp.maximum(s - 1, 0), s > 0, best, bidx)

        def after(dep):
            first = jnp.where(s < 0, dep, hm[NM:NM + 8, 0:128])
            row = jnp.concatenate([first, hm[NM:NM + 8, 128:]], axis=1)
            return jnp.concatenate([hm[:NM], row, hm[NM + 8:]], axis=0)

        t = jnp.maximum(s - 5, 0)
        side = [best, pre(jnp.minimum(s + 1, NSEG - 1)),
                x_tile(jnp.minimum(s // 4 + 2, NG - 1), s % 4), out_tile(t // 4, t % 4)]
        tq = [None] * 4
        for kt in _TILES:
            for n in range(4):
                w = wyq[n // 2, kt * 64:(kt + 1) * 64, (n % 2) * 128:(n % 2 + 1) * 128]
                t1 = _dot(hm[:, kt * 128:(kt + 1) * 128], _unpack(w))
                tq[n] = t1 if tq[n] is None else tq[n] + t1
        for n in range(2, 4):
            t2 = _dot(hm, _unpack(wyq[n]))
            tq += [t2[:, :128], t2[:, 128:]]
        tails = _tail_keys(hq)
        st = []
        for j in range(3):
            for p in range(NP):
                k = j * NP + p
                lhs = after(side[(k - 8) // 4]) if k in (8, 12, 16, 20) else hm
                _project_main(lhs[:, :DM], wym, ys, j, p)
                if k in (2, 4, 6, 9, 11, 13, 15, 17):
                    st.append(_dot(tq[len(st)], tails[len(st)], NT))
        hk = hm[:, :DM]
        for p in range(NP):
            _project_tail(hk, wyt, ys, p, False)
        sc = {}
        for p in range(NP):
            _project_tail(hk, wft, fs, p, True)
            if p in (5, 7):
                sc[len(sc)] = _scores(hq, ys, len(sc))
        for j in range(3):
            for p in range(NP):
                _project_main(hk, wfm, fs, j, p)
                if j == 0 and p in (1, 3, 5):
                    sc[len(sc)] = _scores(hq, ys, len(sc))
        prob = _softmax(_add_tail_scores(sc, st))
        o = {j: _attend(prob, fs, j) for j in _TILES[:2]}
        u = jnp.concatenate([_dot(l, tails[p]) for p, l in enumerate(_slot_probs(prob))], axis=1)
        o.update({j: _attend(prob, fs, j) for j in _TILES[2:]})
        o = {j: o[j] + _dot(u, _unpack(wfu[j])) for j in _TILES}
        o = jnp.concatenate([o[j] for j in range(4)], axis=1)
        obuf[...] = o[NM:]
        return o[:NM], best, bidx

    init = (_widen(mem0_ref[...].astype(F32)),
            jnp.full((8, 128), -jnp.inf, F32), jnp.zeros((8, 128), jnp.int32))

    def steps(i, carry):
        pl.when(i * _UNROLL == 8)(lambda: arrive("x", 2))
        pl.when(i * _UNROLL == s_early)(early.start)
        for u in range(_UNROLL):
            carry = step(i * _UNROLL + u, carry)
        return carry

    _, best, bidx = lax.fori_loop(0, NSEG // _UNROLL, steps, init)
    arrive("w", 1)
    best, bidx = post(NSEG - 1, True, best, bidx)
    rest = pl.ds(n_early * 128, S - n_early * 128)
    last = copy(_NSEM - 2, outT_v.at[pl.ds(0, D), rest], out_hbm.at[:, rest])
    out_tile(NG - 2, 3)
    for j in range(4):
        out_tile(NG - 1, j)
    last.start()
    early.wait()

    top = jnp.max(best, axis=0, keepdims=True)
    idx = jnp.min(jnp.where(best == top, bidx, S - 1))
    sel = jnp.broadcast_to(h2tok[pl.ds(idx, 1), :], (8, DP))[:, :D]
    gate = _dot(sel, wg_v[...])
    act = gate * jax.nn.sigmoid(gate) * _dot(sel, wu_v[...])
    y = _widen(_dot(act, wd_v[...], NT)) * jax.nn.sigmoid(top[:, 0:1])
    ztok[pl.ds(idx, 1), :] = ztok[pl.ds(idx, 1), :] + (vec[5] * y)[0:1]

    top_g = idx // 128
    cols = pl.ds(pl.multiple_of(top_g * 128, 128), 128)
    patch = copy(_NSEM - 1, outT_v.at[pl.ds(0, D), cols], out_hbm.at[:, cols])
    last.wait()
    for j in range(4):
        out_tile(top_g, j)
    patch.start()
    patch.wait()


@functools.partial(jax.jit, static_argnames=("A_seg_len",))
def pallas_adaLN_cond__memory_aug_recurrent_mem_tr__moe_arch_mod__prompt_kernel(
    A_x: jax.Array,
    A_mem0: jax.Array,
    A_Wq: jax.Array,
    A_Wk: jax.Array,
    A_Wv: jax.Array,
    A_Wo: jax.Array,
    A_seg_len: int,
    B_x: jax.Array,
    B_w_r: jax.Array,
    B_w_gate: jax.Array,
    B_w_up: jax.Array,
    B_w_down: jax.Array,
    c: jax.Array,
    w_mod: jax.Array,
):
    del B_x
    assert A_seg_len == SEG and A_x.shape == (1, S, D) and A_Wq.shape == (D, NH, DH)
    hbm = pl.BlockSpec(memory_space=pl.ANY)
    split = pltpu.VMEM((2, D * NH, 128), BF16)
    wmain = pltpu.VMEM((3, NP, DM // 2, 256), U32)
    wtail = pltpu.VMEM((NP, DM // 2, 128), U32)
    stack = pltpu.VMEM((NB * 64, DP), U32)
    tok = pltpu.VMEM((S, DP), F32)
    ff = pltpu.VMEM((D, FF), BF16)
    outT = pl.pallas_call(
        _kernel,
        out_shape=jax.ShapeDtypeStruct((D, S), BF16),
        in_specs=[hbm] * 12,
        out_specs=hbm,
        scratch_shapes=[
            pltpu.VMEM((DP, S), BF16), split, split, split, pltpu.VMEM((NH, D, DH), BF16),
            pltpu.VMEM((D, 6 * D), BF16), ff, ff, ff,
            wmain, wtail, pltpu.VMEM((NP // 2, DP // 2, 256), U32),
            wmain, wtail, pltpu.VMEM((4, NP * 64, 128), U32), stack, stack,
            pltpu.VMEM((7, 8, DP), F32),
            tok, pltpu.VMEM((SEG, DP), F32), pltpu.VMEM((SEG, DP), F32), tok, tok,
            pltpu.VMEM((DP, S), BF16),
            pltpu.VMEM((NM, D), BF16), pltpu.VMEM((D,), BF16), pltpu.VMEM((1, D), BF16),
            pltpu.SemaphoreType.DMA((_NSEM,)),
        ],
        compiler_params=pltpu.CompilerParams(vmem_limit_bytes=100 * 1024 * 1024),
    )(
        A_x[0].T, A_mem0[0],
        A_Wq.reshape(D * NH, DH), A_Wk.reshape(D * NH, DH), A_Wv.reshape(D * NH, DH),
        A_Wo.transpose(0, 2, 1), B_w_r, B_w_gate, B_w_up, B_w_down.T, c, w_mod,
    )
    return outT.T[None]
```

```python
import functools

import jax
import jax.numpy as jnp
from jax import lax
import jax.experimental.pallas as pl
import jax.experimental.pallas.tpu as pltpu

D = 448
DM = 384
DT = D - DM
DP = 512
NH = 16
NP = NH // 2
DH = 256
NM = 8
SEG = 32
NB = (NM + SEG) // 8
S = 2048
NSEG = S // SEG
NG = S // 128
FF = 1792
EPS = 1e-5
SCALE = DH ** -0.5

_EDGES = (0, 128, 256, DM, D)
_GROUPS = [[("w" + t[0], int(t[1])) for t in g.split()] for g in
           "o0 v0|v1|o1|v3|o2|o3|o4 o5|o6 o7|v2|q0 k0|q1|k1|q3 k3|q2|k2".split("|")]
_ARRIVALS = tuple(a for g in _GROUPS for a in g) + (
    ("w", 0), ("x", 0), ("x", 1), ("x", 2), ("w", 1))
_AHEAD = 8
_NSEM = sum({"wo": 1, "w": 4}.get(k, 2) for k, _ in _ARRIVALS) + 3

_UNROLL = 4
_TILES = (3, 0, 1, 2)

F32 = jnp.float32
BF16 = jnp.bfloat16
U32 = jnp.uint32
NN = (((1,), (0,)), ((), ()))
NT = (((1,), (1,)), ((), ()))


def _dot(a, b, dims=NN):
    return lax.dot_general(a, b, dims, preferred_element_type=F32)


def _pack(x):
    return pltpu.bitcast(x.astype(BF16), U32)


def _unpack(x):
    return pltpu.bitcast(x, BF16)


def _lane(shape):
    return lax.broadcasted_iota(jnp.int32, shape, 1)


def _widen(v):
    t = v[:, DM:D]
    return jnp.concatenate([v[:, :DM], t, t], axis=1)


def _feat_sum(v):
    head = _lane((v.shape[0], 128)) < DT
    acc = v[:, 0:128] + v[:, 128:256] + v[:, 256:384] + jnp.where(head, v[:, 384:512], 0.0)
    return jnp.sum(acc, axis=1, keepdims=True)


def _norm_mod(v, scale1, shift):
    xc = v - _feat_sum(v) * (1.0 / D)
    var = _feat_sum(xc * xc) * (1.0 / D)
    return xc * lax.rsqrt(var + EPS) * scale1 + shift


def _group8(x, op):
    lane = _lane(x.shape)
    for size, step in ((4, 1), (8, 4)):
        pos = lane & (size - 1)
        x = functools.reduce(op, [x] + [
            jnp.where(pos >= d, pltpu.roll(x, d, 1), pltpu.roll(x, 128 + d - size, 1))
            for d in range(step, size, step)])
    return x


def _head_pair(buf, p, i):
    rows = pl.ds(_EDGES[i] * NP + p, _EDGES[i + 1] - _EDGES[i], stride=NP)
    u = jnp.concatenate([buf.at[t].bitcast(U32)[rows, :] for t in range(2)], axis=1)
    lo = pltpu.bitcast(u << 16, F32)
    hi = pltpu.bitcast(u & jnp.uint32(0xFFFF0000), F32)
    return lo, hi


def _merge_tail(lhs_tail, rhs, scale):
    pad = [jnp.zeros((128 - rhs[0].shape[0], DH), BF16)] if rhs[0].shape[0] < 128 else []
    a = jnp.concatenate(
        [_dot(lhs_tail[h], jnp.concatenate([rhs[h].astype(BF16)] + pad, axis=0), NT)
         for h in range(2)], axis=0)
    return _pack((a if scale == 1.0 else a * scale).T)


def _project_main(hm, wm_ref, st_ref, j, p):
    y = _dot(hm, _unpack(wm_ref[j, p]))
    for kb in range(NB):
        r = y[kb * 8:(kb + 1) * 8]
        blk = jnp.concatenate([r[:, :128], r[:, 128:]], axis=0)
        st_ref[kb * 64 + p * 8:kb * 64 + p * 8 + 8, j * 128:(j + 1) * 128] = _pack(blk)


def _project_tail(hm, wt_ref, st_ref, p, dup):
    head = _lane((8, 128)) < DT
    y = _dot(hm, _unpack(wt_ref[p]))
    other = pltpu.roll(y, DT, 1) if dup else jnp.zeros_like(y)
    for kb in range(NB):
        r, o = y[kb * 8:(kb + 1) * 8], other[kb * 8:(kb + 1) * 8]
        blk = jnp.concatenate([jnp.where(head, r, o), jnp.where(head, o, r)], axis=0)
        st_ref[kb * 64 + p * 8:kb * 64 + p * 8 + 8, DM:DP] = _pack(blk)


def _seeing(kb):
    return [0] + list(range(max(kb, 1), NB))


def _scores(hq, ys_ref, yt_ref, kb):
    qbs = _seeing(kb)
    yt_ref[kb] = pltpu.bitcast(_unpack(ys_ref[kb * 64:(kb + 1) * 64, :]).T, U32)
    sc = _dot(jnp.concatenate([hq[q] for q in qbs], axis=0), _unpack(yt_ref[kb]))
    return {q: sc[i * 8:(i + 1) * 8] for i, q in enumerate(qbs)}


def _tail_keys(hq):
    head = _lane((8, 128)) < DT
    blk = [jnp.concatenate([jnp.where(head, t[:, DM:], 0.0), jnp.where(head, 0.0, t[:, DM:])],
                           axis=0).astype(BF16) for t in hq]
    blk += [jnp.zeros((16, 128), BF16)] * (NP - NB)
    return [jnp.concatenate([blk[(i - p) % NP] for i in range(NP)], axis=0) for p in range(NP)]


def _add_tail_scores(sc, st):
    slot = _lane((8, 128)) // 16
    out = {}
    for kb in range(NB):
        out[kb] = {}
        for qb in sc[kb]:
            g = st[0][qb * 8:(qb + 1) * 8]
            for p in range(1, NP):
                g = jnp.where(slot == (p + kb) % NP, st[p][qb * 8:(qb + 1) * 8], g)
            out[kb][qb] = sc[kb][qb] + (pltpu.roll(g, 128 - 16 * kb, 1) if kb else g)
    return out


def _slot_probs(prob):
    slot = _lane((8, 128)) // 16
    rot = [{kb: pltpu.roll(t, 16 * kb, 1) if kb else t for kb, t in r.items()} for r in prob]
    out = []
    for p in range(NP):
        rows = []
        for r in rot:
            g = r[0] if len(r) == NB else jnp.where(slot == p, r[0], 0.0)
            for kb in range(1, len(r)):
                g = jnp.where(slot == (p + kb) % NP, r[kb], g)
            rows.append(g)
        out.append(jnp.concatenate(rows, axis=0))
    return out


def _softmax(sc):
    tri = (_lane((8, 128)) & 7) <= lax.broadcasted_iota(jnp.int32, (8, 128), 0)
    vis = [{kb: jnp.where(tri, sc[kb][qb], -1e9) if 0 < qb == kb else sc[kb][qb]
            for kb in range(NB) if qb in sc[kb]} for qb in range(NB)]
    mx = _group8(jnp.concatenate(
        [functools.reduce(jnp.maximum, r.values()) for r in vis], axis=0), jnp.maximum)
    ex = [{kb: jnp.exp(t - mx[qb * 8:(qb + 1) * 8]) for kb, t in r.items()}
          for qb, r in enumerate(vis)]
    den = _group8(jnp.concatenate(
        [functools.reduce(jnp.add, r.values()) for r in ex], axis=0), jnp.add)
    inv = 1.0 / den
    return [{kb: t * inv[qb * 8:(qb + 1) * 8] for kb, t in r.items()} for qb, r in enumerate(ex)]


def _attend(prob, fs_ref, j):
    acc = [None] * NB
    for kb in range(NB):
        qbs = _seeing(kb)
        o = _dot(jnp.concatenate([prob[q][kb] for q in qbs], axis=0),
                 _unpack(fs_ref[kb * 64:(kb + 1) * 64, j * 128:(j + 1) * 128]))
        for i, q in enumerate(qbs):
            t = o[i * 8:(i + 1) * 8]
            acc[q] = t if acc[q] is None else acc[q] + t
    return jnp.concatenate(acc, axis=0)


def _kernel(xT_hbm, mem0_hbm, wq_hbm, wk_hbm, wv_hbm, woT_hbm, wr_hbm, wg_hbm, wu_hbm, wdT_hbm,
            c_hbm, wmod_hbm, out_hbm,
            xT_v, wq_v, wk_v, wv_v, woT_v, wmod_v, wg_v, wu_v, wd_v,
            wym, wyt, wyq, wfm, wft, wfu, ys, fs, vec, xtok, hbuf, obuf, h2tok, ztok, outT_v,
            mem0_ref, wr_ref, c_ref, wk_d, wq_d, yt, sems):
    def copy(i, src, dst):
        return pltpu.make_async_copy(src, dst, sems.at[i])

    plan = []
    for kind, i in _ARRIVALS:
        if kind == "wo":
            pairs = [(woT_hbm.at[pl.ds(2 * i, 2)], woT_v.at[pl.ds(2 * i, 2)])]
        elif kind in ("wv", "wq", "wk"):
            src, dst = {"wv": (wv_hbm, wv_v), "wq": (wq_hbm, wq_v), "wk": (wk_hbm, wk_v)}[kind]
            r = pl.ds(_EDGES[i] * NH, (_EDGES[i + 1] - _EDGES[i]) * NH)
            pairs = [(src.at[r, pl.ds(t * 128, 128)], dst.at[t, r]) for t in range(2)]
        elif kind == "x":
            cols = pl.ds(*((0, 256), (256, 256), (512, S - 512))[i])
            pairs = [(xT_hbm.at[:, cols], xT_v.at[pl.ds(0, D), cols]),
                     (xT_hbm.at[pl.ds(DM, DT), cols], xT_v.at[pl.ds(D, DT), cols])]
        else:
            pairs = [[(mem0_hbm, mem0_ref), (wr_hbm, wr_ref), (c_hbm, c_ref), (wmod_hbm, wmod_v)],
                     [(wg_hbm, wg_v), (wu_hbm, wu_v), (wdT_hbm, wd_v)]][i]
        first = sum(len(c) for c in plan)
        plan.append([copy(first + n, a, b) for n, (a, b) in enumerate(pairs)])
    started = 0

    def arrive(kind, i):
        nonlocal started
        n = _ARRIVALS.index((kind, i))
        while started < min(n + 1 + _AHEAD, len(plan)):
            for c in plan[started]:
                c.start()
            started += 1
        for c in plan[n]:
            c.wait()

    for pieces in plan[:_AHEAD]:
        for c in pieces:
            c.start()
    started = _AHEAD

    obuf[...] = jnp.zeros(obuf.shape, F32)
    ztok[0:128, :] = jnp.zeros((128, DP), F32)

    def merge_f(p, i):
        v, rows = _head_pair(wv_v, p, i), slice(i * 64, (i + 1) * 64)
        wo = [woT_v[2 * p + h, 0:DM, :] for h in range(2)]
        wo_tail = [woT_v[2 * p + h, DM:D, :] for h in range(2)]
        for h in range(2):
            if i < 3:
                a = _dot(v[h], wo[h], NT)
                for j in range(3):
                    wfm[j, p, rows, h * 128:(h + 1) * 128] = _pack(a[:, j * 128:(j + 1) * 128])
            else:
                a = _dot(v[h], jnp.concatenate([wo[h], wo_tail[h], wo_tail[h]], axis=0), NT)
                for j in range(4):
                    wfu[j, p * 64 + h * 32:p * 64 + h * 32 + 32, :] = _pack(
                        a[:, j * 128:(j + 1) * 128])
        if i < 3:
            wft[p, rows, :] = _merge_tail(wo_tail, v, 1.0)

    seen = {}

    def heads(buf, dst, p, i):
        rows, key = slice(_EDGES[i] // 2, _EDGES[i + 1] // 2), (id(dst), p, i)
        if key not in seen:
            seen[key] = [t.astype(BF16) for t in _head_pair(buf, p, i)]
            for h in range(2):
                dst[2 * p + h, rows, :] = pltpu.bitcast(seen[key][h], U32)
        return seen[key] or [_unpack(dst[2 * p + h, rows, :]) for h in range(2)]

    def merge_y(p, i, j):
        k, q = heads(wk_v, wk_d, p, i), heads(wq_v, wq_d, p, j)
        if i == 3:
            wyq[p // 2, j * 64:(j + 1) * 64, (p % 2) * 128:(p % 2 + 1) * 128] = _merge_tail(
                k, q, SCALE)
        elif j == 3:
            wyt[p, i * 64:(i + 1) * 64, :] = _merge_tail(q, k, SCALE)
        else:
            for h in range(2):
                wym[j, p, i * 64:(i + 1) * 64, h * 128:(h + 1) * 128] = _pack(
                    _dot(k[h], q[h], NT) * SCALE)

    def rows(i):
        return jnp.concatenate([vec[i]] * (SEG // 8), axis=0)

    def x_tile(g, j):
        g0, j0 = pl.multiple_of(g * 128, 128), pl.multiple_of(j * 128, 128)
        t = xT_v[pl.ds(j0, 128), pl.ds(g0, 128)].astype(F32).T
        xtok[pl.ds(g0, 128), pl.ds(j0, 128)] = t
        return t[120:128]

    def out_tile(g, j):
        g0, j0 = pl.multiple_of(g * 128, 128), pl.multiple_of(j * 128, 128)
        t = ztok[pl.ds(g0, 128), pl.ds(j0, 128)].T
        outT_v[pl.ds(j0, 128), pl.ds(g0, 128)] = t.astype(BF16)
        return t[120:128]

    def seg_rows(s):
        return pl.ds(pl.multiple_of(s * SEG, SEG), SEG)

    def pre(s):
        h = _norm_mod(xtok[seg_rows(s), :], rows(1), rows(0))
        hbuf[...] = h
        return functools.reduce(jnp.maximum, [h[b * 8:(b + 1) * 8, 0:128] for b in range(SEG // 8)])

    def post(s, live, best, bidx):
        x1 = xtok[seg_rows(s), :] + rows(2) * obuf[...]
        h2 = _norm_mod(x1, rows(4), rows(3))
        h2tok[seg_rows(s), :] = h2
        ztok[seg_rows(s), :] = x1 + rows(5) * h2
        r = _feat_sum(h2 * rows(6))
        sub = lax.broadcasted_iota(jnp.int32, (8, 128), 0)
        for b in range(SEG // 8):
            rb = jnp.broadcast_to(r[b * 8:(b + 1) * 8], (8, 128))
            better = jnp.logical_and(rb > best, live)
            best = jnp.where(better, rb, best)
            bidx = jnp.where(better, sub + (s * SEG + b * 8), bidx)
        return best, bidx

    def setup():
        arrive("w", 0)
        arrive("x", 0)
        cv = jnp.broadcast_to(c_ref[...].astype(F32), (8, D))
        mod = _dot(cv * jax.nn.sigmoid(cv), wmod_v[...])
        for i in range(6):
            v = _widen(mod[:, i * D:(i + 1) * D])
            vec[i] = v + 1.0 if i in (1, 4) else v
        vec[6] = _widen(jnp.broadcast_to(wr_ref[...].astype(F32).reshape(1, D), (8, D)))
        for g in range(2):
            for j in range(4):
                x_tile(g, j)
        pre(0)

    have = []
    for group in _GROUPS:
        for piece in group:
            arrive(*piece)
        have += group
        seen = dict.fromkeys(seen)

        def fresh(a, b):
            return a in have and b in have and (a in group or b in group)

        for p in range(NP):
            if group is _GROUPS[-1] and p == 6:
                setup()
            for i in range(4):
                if fresh(("wv", i), ("wo", p)):
                    merge_f(p, i)
                for j in range(4):
                    if fresh(("wk", i), ("wq", j)):
                        merge_y(p, i, j)

    arrive("x", 1)
    s_early = NSEG - _UNROLL
    n_early = (s_early - 9) // 4 + 1
    early = copy(_NSEM - 3, outT_v.at[pl.ds(0, D), pl.ds(0, n_early * 128)],
                 out_hbm.at[:, pl.ds(0, n_early * 128)])

    def step(s, carry):
        mem, best, bidx = carry
        hm = jnp.concatenate([mem, hbuf[...]], axis=0)
        hq = [hm[q * 8:(q + 1) * 8] for q in range(NB)]
        best, bidx = post(jnp.maximum(s - 1, 0), s > 0, best, bidx)

        def after(dep):
            first = jnp.where(s < 0, dep, hm[NM:NM + 8, 0:128])
            row = jnp.concatenate([first, hm[NM:NM + 8, 128:]], axis=1)
            return jnp.concatenate([hm[:NM], row, hm[NM + 8:]], axis=0)

        t = jnp.maximum(s - 5, 0)
        side = [best, pre(jnp.minimum(s + 1, NSEG - 1)),
                x_tile(jnp.minimum(s // 4 + 2, NG - 1), s % 4), out_tile(t // 4, t % 4)]
        tq = [None] * 4
        for kt in _TILES:
            for n in range(4):
                w = wyq[n // 2, kt * 64:(kt + 1) * 64, (n % 2) * 128:(n % 2 + 1) * 128]
                t1 = _dot(hm[:, kt * 128:(kt + 1) * 128], _unpack(w))
                tq[n] = t1 if tq[n] is None else tq[n] + t1
        for n in range(2, 4):
            t2 = _dot(hm, _unpack(wyq[n]))
            tq += [t2[:, :128], t2[:, 128:]]
        tails = _tail_keys(hq)
        st = []
        for j in range(3):
            for p in range(NP):
                k = j * NP + p
                lhs = after(side[(k - 8) // 4]) if k in (8, 12, 16, 20) else hm
                _project_main(lhs[:, :DM], wym, ys, j, p)
                if k in (2, 4, 6, 9, 11, 13, 15, 17):
                    st.append(_dot(tq[len(st)], tails[len(st)], NT))
        hk = hm[:, :DM]
        for p in range(NP):
            _project_tail(hk, wyt, ys, p, False)
        for p in range(NP):
            _project_tail(hk, wft, fs, p, True)
        sc = {}
        for j in range(3):
            for p in range(NP):
                _project_main(hk, wfm, fs, j, p)
                if j == 0 and 2 <= p < 2 + NB:
                    sc[p - 2] = _scores(hq, ys, yt, p - 2)
        prob = _softmax(_add_tail_scores(sc, st))
        u = jnp.concatenate([_dot(l, tails[p]) for p, l in enumerate(_slot_probs(prob))], axis=1)
        o = {j: _attend(prob, fs, j) for j in _TILES}
        o = {j: o[j] + _dot(u, _unpack(wfu[j])) for j in _TILES}
        o = jnp.concatenate([o[j] for j in range(4)], axis=1)
        obuf[...] = o[NM:]
        return o[:NM], best, bidx

    init = (_widen(mem0_ref[...].astype(F32)),
            jnp.full((8, 128), -jnp.inf, F32), jnp.zeros((8, 128), jnp.int32))

    def steps(i, carry):
        pl.when(i * _UNROLL == 8)(lambda: arrive("x", 2))
        pl.when(i * _UNROLL == s_early)(early.start)
        for u in range(_UNROLL):
            carry = step(i * _UNROLL + u, carry)
        return carry

    _, best, bidx = lax.fori_loop(0, NSEG // _UNROLL, steps, init)
    arrive("w", 1)
    best, bidx = post(NSEG - 1, True, best, bidx)

    rest = pl.ds(n_early * 128, S - n_early * 128)
    last = copy(_NSEM - 2, outT_v.at[pl.ds(0, D), rest], out_hbm.at[:, rest])
    out_tile(NG - 2, 3)
    for j in range(4):
        out_tile(NG - 1, j)
    last.start()
    early.wait()

    top = jnp.max(best, axis=0, keepdims=True)
    idx = jnp.min(jnp.where(best == top, bidx, S - 1))
    sel = jnp.broadcast_to(h2tok[pl.ds(idx, 1), :], (8, DP))[:, :D]
    gate = _dot(sel, wg_v[...])
    act = gate * jax.nn.sigmoid(gate) * _dot(sel, wu_v[...])
    y = _widen(_dot(act, wd_v[...], NT)) * jax.nn.sigmoid(top[:, 0:1])
    ztok[pl.ds(idx, 1), :] = ztok[pl.ds(idx, 1), :] + (vec[5] * y)[0:1]

    top_g = idx // 128
    cols = pl.ds(pl.multiple_of(top_g * 128, 128), 128)
    patch = copy(_NSEM - 1, outT_v.at[pl.ds(0, D), cols], out_hbm.at[:, cols])
    last.wait()
    for j in range(4):
        out_tile(top_g, j)
    patch.start()
    patch.wait()


@functools.partial(jax.jit, static_argnames=("A_seg_len",))
def pallas_adaLN_cond__memory_aug_recurrent_mem_tr__moe_arch_mod__prompt_kernel(
    A_x: jax.Array,
    A_mem0: jax.Array,
    A_Wq: jax.Array,
    A_Wk: jax.Array,
    A_Wv: jax.Array,
    A_Wo: jax.Array,
    A_seg_len: int,
    B_x: jax.Array,
    B_w_r: jax.Array,
    B_w_gate: jax.Array,
    B_w_up: jax.Array,
    B_w_down: jax.Array,
    c: jax.Array,
    w_mod: jax.Array,
):
    del B_x
    assert A_seg_len == SEG and A_x.shape == (1, S, D) and A_Wq.shape == (D, NH, DH)
    hbm = pl.BlockSpec(memory_space=pl.ANY)
    split = pltpu.VMEM((2, D * NH, 128), BF16)
    wmain = pltpu.VMEM((3, NP, DM // 2, 256), U32)
    wtail = pltpu.VMEM((NP, DM // 2, 128), U32)
    stack = pltpu.VMEM((NB * 64, DP), U32)
    tok = pltpu.VMEM((S, DP), F32)
    ff = pltpu.VMEM((D, FF), BF16)
    outT = pl.pallas_call(
        _kernel,
        out_shape=jax.ShapeDtypeStruct((D, S), BF16),
        in_specs=[hbm] * 12,
        out_specs=hbm,
        scratch_shapes=[
            pltpu.VMEM((DP, S), BF16), split, split, split, pltpu.VMEM((NH, D, DH), BF16),
            pltpu.VMEM((D, 6 * D), BF16), ff, ff, ff,
            wmain, wtail, pltpu.VMEM((NP // 2, DP // 2, 256), U32),
            wmain, wtail, pltpu.VMEM((4, NP * 64, 128), U32), stack, stack,
            pltpu.VMEM((7, 8, DP), F32),
            tok, pltpu.VMEM((SEG, DP), F32), pltpu.VMEM((SEG, DP), F32), tok, tok,
            pltpu.VMEM((DP, S), BF16),
            pltpu.VMEM((NM, D), BF16), pltpu.VMEM((D,), BF16), pltpu.VMEM((1, D), BF16),
            pltpu.VMEM((NH, D // 2, DH), U32), pltpu.VMEM((NH, D // 2, DH), U32),
            pltpu.VMEM((NB, DP // 2, 128), U32), pltpu.SemaphoreType.DMA((_NSEM,)),
        ],
        compiler_params=pltpu.CompilerParams(vmem_limit_bytes=100 * 1024 * 1024),
    )(
        A_x[0].T, A_mem0[0],
        A_Wq.reshape(D * NH, DH), A_Wk.reshape(D * NH, DH), A_Wv.reshape(D * NH, DH),
        A_Wo.transpose(0, 2, 1), B_w_r, B_w_gate, B_w_up, B_w_down.T, c, w_mod,
    )
    return outT.T[None]
```
